```python
import os as _os
_os.environ.setdefault("JAX_PLATFORMS", "cpu")
import jax
import jax.numpy as jnp

def _softmax(x, axis=-1):
    return jax.nn.softmax(x, axis=axis)
def _gelu(x):
    return jax.nn.gelu(x, approximate=True)
def _silu(x):
    return jax.nn.silu(x)
def _sigmoid(x):
    return jax.nn.sigmoid(x)
def _layernorm(x, axis=-1, eps=1e-5):
    m = jnp.mean(x, axis=axis, keepdims=True)
    v = jnp.var(x, axis=axis, keepdims=True)
    return (x - m) / jnp.sqrt(v + eps)
def _scatter_add(tgt, idx, src, axis=0):
    return tgt.at[idx].add(src)
def _segment_sum(src, seg, n):
    return jax.ops.segment_sum(src, seg, n)
class _Rng:
    def __init__(self, key):
        self._k = key
    def _next(self):
        self._k, sub = jax.random.split(self._k)
        return sub
    def normal(self, shape):
        return jax.random.normal(self._next(), shape, dtype=jnp.bfloat16)
    def randint(self, lo, hi, shape):
        return jax.random.randint(self._next(), shape, lo, hi, dtype=jnp.int32)
    def uniform(self, shape, lo=0.0, hi=1.0):
        return jax.random.uniform(self._next(), shape, jnp.bfloat16, lo, hi)
    def permutation(self, n):
        return jax.random.permutation(self._next(), n)


kernel_name = 'concat_heads__gqa_block_cached__sliding_block_cached__decode'

def setup_inputs():
    _rng = _Rng(jax.random.key(int.from_bytes(__import__("os").urandom(4), "little")))
    _w = (lambda a: (lambda t: t.astype(jnp.bfloat16) if jnp.issubdtype(t.dtype, jnp.floating) else t)(jnp.asarray(a)))
    def _A_setup():
        B, Sq, D = 2, 1, 448
        Hq, Hkv, Sk, Dh = 16, 8, 8192, 256
        assert Hq % Hkv == 0, (Hq, Hkv)
        return {
            "x": _w((lambda *s: _rng.normal(s) * 0.8)(B, Sq, D)),
            "k_cache": _w((lambda *s: _rng.normal(s) * 0.8)(B, Hkv, Sk, Dh)),
            "v_cache": _w((lambda *s: _rng.normal(s) * 0.05)(B, Hkv, Sk, Dh)),
            "wq": _w((lambda *s: _rng.normal(s) * 0.8)(D, Hq * Dh) * (D ** -0.5)),
            "wo": _w((lambda *s: _rng.normal(s) * 0.05)(Hq * Dh, D) * ((Hq * Dh) ** -0.5)),
        }
    _A_in = _A_setup()

    def _B_setup():
        B, Sq, D = 2, 1, 448
        Hq, Hkv, Sk, Dh = 16, 8, 8192, 256
        assert Hq % Hkv == 0, (Hq, Hkv)
        return {
            "x": _w((lambda *s: _rng.normal(s) * 0.8)(B, Sq, D)),
            "k_cache": _w((lambda *s: _rng.normal(s) * 0.8)(B, Hkv, Sk, Dh)),
            "v_cache": _w((lambda *s: _rng.normal(s) * 0.05)(B, Hkv, Sk, Dh)),
            "wq": _w((lambda *s: _rng.normal(s) * 0.8)(D, Hq * Dh) * (D ** -0.5)),
            "wo": _w((lambda *s: _rng.normal(s) * 0.05)(Hq * Dh, D) * ((Hq * Dh) ** -0.5)),
        }
    _B_in = _B_setup()

    return {
        "A_x": _A_in["x"],
        "A_k_cache": _A_in["k_cache"],
        "A_v_cache": _A_in["v_cache"],
        "A_wq": _A_in["wq"],
        "A_wo": _A_in["wo"],
        "B_x": _B_in["x"],
        "B_k_cache": _B_in["k_cache"],
        "B_v_cache": _B_in["v_cache"],
        "B_wq": _B_in["wq"],
        "B_wo": _B_in["wo"],
    }

def reference(A_x, A_k_cache, A_v_cache, A_wq, A_wo, B_x, B_k_cache, B_v_cache, B_wq, B_wo):
    def _A_ref(x, k_cache, v_cache, wq, wo):
        B, Sq, D = x.shape
        Hq, Dh = 16, 256
        Hkv = k_cache.shape[1]
        rep = Hq // Hkv
        q = (lambda x, *d: x.transpose(*d))((x @ wq).reshape(B, Sq, Hq, Dh), 0, 2, 1, 3)
        k = jnp.repeat(k_cache, rep, axis=1)
        v = jnp.repeat(v_cache, rep, axis=1)
        scores = jnp.einsum("bhqd,bhkd->bhqk", q, k) * (Dh ** -0.5)
        p = _softmax(scores, axis=-1)
        o = jnp.einsum("bhqk,bhkd->bhqd", p, v)
        return (lambda x, *d: x.transpose(*d))(o, 0, 2, 1, 3).reshape(B, Sq, Hq * Dh) @ wo

    def _B_ref(x, k_cache, v_cache, wq, wo):
        B, Sq, D = x.shape
        Hq, Dh = 16, 256
        Hkv, Sk = k_cache.shape[1], k_cache.shape[2]
        W = min(4096, max(256, Sk // 4))
        rep = Hq // Hkv
        q = (lambda x, *d: x.transpose(*d))((x @ wq).reshape(B, Sq, Hq, Dh), 0, 2, 1, 3)
        k = jnp.repeat(k_cache[:, :, Sk - W:, :], rep, axis=1)
        v = jnp.repeat(v_cache[:, :, Sk - W:, :], rep, axis=1)
        scores = jnp.einsum("bhqd,bhkd->bhqk", q, k) * (Dh ** -0.5)
        p = _softmax(scores, axis=-1)
        o = jnp.einsum("bhqk,bhkd->bhqd", p, v)
        return (lambda x, *d: x.transpose(*d))(o, 0, 2, 1, 3).reshape(B, Sq, Hq * Dh) @ wo

    a = _A_ref(A_x, A_k_cache, A_v_cache, A_wq, A_wo)
    b = _B_ref(B_x, B_k_cache, B_v_cache, B_wq, B_wo)
    return jnp.concatenate([a, b], axis=-1)
```

```python
import functools
import jax
import jax.numpy as jnp
from jax import lax
from jax.experimental import pallas as pl
from jax.experimental.pallas import tpu as pltpu

NT = (((1,), (1,)), ((), ()))
NN = (((1,), (0,)), ((), ()))

B, D = 2, 448
HQ, HKV, SK, DH = 16, 8, 8192, 256
REP = HQ // HKV
W = min(4096, max(256, SK // 4))
F = HQ * DH


def make_kernel(CH=2048, NB=3, tail_cols=(256, 128, 128), kprio=0, vprio=0):
    NCA = SK // CH
    NCB = W // CH
    NA = B * HKV * NCA
    NBs = B * HKV * NCB
    NSTEP = NA + NBs
    tail_total = sum(tail_cols)
    head_cols = F - tail_total
    assert tail_total == 512

    def kernel(ax, ak, av, awq, awoT, bx, bk, bv, bwq, bwoT, o_ref,
               kbuf, vbuf, wq_buf, wo_buf, x_buf, x8_s, q_s, o_s, outa_s,
               ksem, vsem, wsem):
        def kv_copy(phase, src, buf, sem, j, slot):
            nc = NCA if phase == 0 else NCB
            c = j % nc
            hb = j // nc
            b = hb % B
            h = hb // B
            base = 0 if phase == 0 else SK - W
            row = pl.multiple_of(base + c * CH, CH)
            return pltpu.make_async_copy(src.at[b, h, pl.ds(row, CH), :], buf.at[slot], sem.at[slot])

        def start_kv(which, i, slot):
            srcs = (ak, bk) if which == "k" else (av, bv)
            buf, sem, prio = (kbuf, ksem, kprio) if which == "k" else (vbuf, vsem, vprio)
            if isinstance(i, int):
                if i < NA:
                    kv_copy(0, srcs[0], buf, sem, i, slot).start(priority=prio)
                elif i < NSTEP:
                    kv_copy(1, srcs[1], buf, sem, i - NA, slot).start(priority=prio)
                return
            @pl.when(i < NA)
            def _():
                kv_copy(0, srcs[0], buf, sem, i, slot).start(priority=prio)
            @pl.when(jnp.logical_and(i >= NA, i < NSTEP))
            def _():
                kv_copy(1, srcs[1], buf, sem, i - NA, slot).start(priority=prio)

        def wait_kv(which, slot):
            buf, sem = (kbuf, ksem) if which == "k" else (vbuf, vsem)
            pltpu.make_async_copy(buf.at[slot], buf.at[slot], sem.at[slot]).wait()

        cp_wqa = pltpu.make_async_copy(awq, wq_buf.at[0], wsem.at[0])
        cp_wqb = pltpu.make_async_copy(bwq, wq_buf.at[1], wsem.at[1])
        cp_xa = pltpu.make_async_copy(ax, x_buf.at[0], wsem.at[2])
        cp_xb = pltpu.make_async_copy(bx, x_buf.at[1], wsem.at[3])
        cp_woa = pltpu.make_async_copy(awoT, wo_buf.at[0], wsem.at[4])
        cp_wob_head = pltpu.make_async_copy(bwoT.at[:, pl.ds(0, head_cols)], wo_buf.at[1, :, pl.ds(0, head_cols)], wsem.at[5])
        cp_wob_tail = []
        off = head_cols
        for t, w in enumerate(tail_cols):
            cp_wob_tail.append((off, w, pltpu.make_async_copy(bwoT.at[:, pl.ds(off, w)], wo_buf.at[1, :, pl.ds(off, w)], wsem.at[6 + t])))
            off += w

        cp_wqa.start()
        cp_xa.start()
        cp_xb.start()
        cp_wqb.start()
        for s in range(NB):
            start_kv("k", s, s)
            start_kv("v", s, s)
        cp_woa.start()
        cp_wob_head.start()

        q_s[...] = jnp.zeros(q_s.shape, q_s.dtype)
        o_s[...] = jnp.zeros(o_s.shape, o_s.dtype)
        x8_s[...] = jnp.zeros(x8_s.shape, x8_s.dtype)
        cp_xa.wait()
        cp_xb.wait()
        for ph in range(2):
            x8_s[ph, 0:B, :] = x_buf[ph].astype(jnp.float32)
        for ph, cp in ((0, cp_wqa), (1, cp_wqb)):
            cp.wait()
            x8 = x8_s[ph].astype(jnp.bfloat16)
            q_all = lax.dot_general(x8, wq_buf[ph], NN, preferred_element_type=jnp.float32)
            q_all = q_all.astype(jnp.bfloat16).astype(jnp.float32) * (DH ** -0.5)
            for h in range(HKV):
                for b in range(B):
                    for r in range(REP):
                        col = (h * REP + r) * DH
                        q_s[ph * HKV * B + h * B + b, r:r + 1, :] = q_all[b:b + 1, col:col + DH]

        def step(i, phase, j, carry):
            m, l, acc = carry
            nc = NCA if phase == 0 else NCB
            c = j % nc
            hb = j // nc
            slot = i % NB
            q = q_s[phase * HKV * B + hb].astype(jnp.bfloat16)
            if nc > 1:
                first = c == 0
                m = jnp.where(first, -jnp.inf, m)
                l = jnp.where(first, 0.0, l)
                acc = jnp.where(first, 0.0, acc)
            wait_kv("k", slot)
            s = lax.dot_general(q, kbuf[slot], NT, preferred_element_type=jnp.float32)
            start_kv("k", i + NB, slot)
            m_cur = jnp.max(s, axis=-1, keepdims=True)
            if nc > 1:
                m_new = jnp.maximum(m, m_cur)
                alpha = jnp.exp(m - m_new)
            else:
                m_new = m_cur
            p = jnp.exp(s - m_new)
            l_cur = jnp.sum(p, axis=-1, keepdims=True)
            wait_kv("v", slot)
            pv = lax.dot_general(p.astype(jnp.bfloat16), vbuf[slot], NN, preferred_element_type=jnp.float32)
            start_kv("v", i + NB, slot)
            def start_tail():
                for _, _, cp in cp_wob_tail:
                    cp.start()
            if isinstance(i, int):
                if i + NB == NSTEP - 1:
                    start_tail()
            elif phase == 1:
                pl.when(i + NB == NSTEP - 1)(start_tail)
            if nc > 1:
                l = alpha * l + l_cur
                acc = alpha * acc + pv
            else:
                l, acc = l_cur, pv

            def fin():
                o = acc / l
                b = hb % B
                h = hb // B
                for r in range(REP):
                    o_s[phase, h * REP + r, pl.ds(b, 1), :] = o[r:r + 1, :]
            if nc > 1:
                pl.when(c == nc - 1)(fin)
            else:
                fin()
            return m_new, l, acc

        def oproj(phase, c0, c1):
            res = None
            c = c0
            while c < c1:
                hq = c // DH
                lo = c - hq * DH
                hi = min(DH, c1 - hq * DH)
                lhs = o_s[phase, hq, :, lo:hi].astype(jnp.bfloat16)
                part = lax.dot_general(lhs, wo_buf[phase, :, c:hq * DH + hi], NT, preferred_element_type=jnp.float32)
                res = part if res is None else res + part
                c = hq * DH + hi
            return res

        init = (jnp.full((8, 1), -jnp.inf, jnp.float32), jnp.zeros((8, 1), jnp.float32), jnp.zeros((8, DH), jnp.float32))
        carry = lax.fori_loop(0, NA, lambda i, c: step(i, 0, i, c), init)

        cp_woa.wait()
        outa_s[...] = oproj(0, 0, F)

        NPEEL = 2 * NCB
        assert NSTEP - 1 - NB >= NA
        carry = lax.fori_loop(NA, NSTEP - NPEEL, lambda i, c: step(i, 1, i - NA, c), carry)
        done_oproj = False
        for i in range(NSTEP - NPEEL, NSTEP):
            if i == NSTEP - 2 * NCB:
                cp_wob_head.wait()
                outb = oproj(1, 0, head_cols)
            carry = step(i, 1, i - NA, carry)
        for off, w, cp in cp_wob_tail:
            cp.wait()
            outb = outb + oproj(1, off, off + w)
        o_ref[:, 0:D] = outa_s[0:B, :].astype(o_ref.dtype)
        o_ref[:, D:2 * D] = outb[0:B, :].astype(o_ref.dtype)

    assert NB <= 2 * NCB + 8

    @jax.jit
    def f(A_x, A_k_cache, A_v_cache, A_wq, A_wo, B_x, B_k_cache, B_v_cache, B_wq, B_wo):
        hbm = pl.BlockSpec(memory_space=pltpu.HBM)
        out = pl.pallas_call(
            kernel,
            out_shape=jax.ShapeDtypeStruct((B, 2 * D), jnp.bfloat16),
            in_specs=[hbm] * 10,
            out_specs=pl.BlockSpec(memory_space=pltpu.VMEM),
            scratch_shapes=[
                pltpu.VMEM((NB, CH, DH), jnp.bfloat16),
                pltpu.VMEM((NB, CH, DH), jnp.bfloat16),
                pltpu.VMEM((2, D, F), jnp.bfloat16),
                pltpu.VMEM((2, D, F), jnp.bfloat16),
                pltpu.VMEM((2, B, D), jnp.bfloat16),
                pltpu.VMEM((2, 8, D), jnp.float32),
                pltpu.VMEM((2 * HKV * B, 8, DH), jnp.float32),
                pltpu.VMEM((2, HQ, 8, DH), jnp.float32),
                pltpu.VMEM((8, D), jnp.float32),
                pltpu.SemaphoreType.DMA((NB,)),
                pltpu.SemaphoreType.DMA((NB,)),
                pltpu.SemaphoreType.DMA((6 + len(tail_cols),)),
            ],
            compiler_params=pltpu.CompilerParams(vmem_limit_bytes=100 * 1024 * 1024),
        )(A_x.reshape(B, D), A_k_cache, A_v_cache, A_wq, A_wo.T,
          B_x.reshape(B, D), B_k_cache, B_v_cache, B_wq, B_wo.T)
        return out.reshape(B, 1, 2 * D)
    return f


_impl = make_kernel()


@jax.jit
def pallas_concat_heads__gqa_block_cached__sliding_block_cached__decode_kernel(
    A_x, A_k_cache, A_v_cache, A_wq, A_wo, B_x, B_k_cache, B_v_cache, B_wq, B_wo):
    return _impl(A_x, A_k_cache, A_v_cache, A_wq, A_wo, B_x, B_k_cache, B_v_cache, B_wq, B_wo)
```

```python
import functools
import jax
import jax.numpy as jnp
from jax import lax
from jax.experimental import pallas as pl
from jax.experimental.pallas import tpu as pltpu

NT = (((1,), (1,)), ((), ()))
NN = (((1,), (0,)), ((), ()))

B, D = 2, 448
HQ, HKV, DH = 16, 8, 256
REP = HQ // HKV
F = HQ * DH
LO, HI = 1, 0


def make_kernel(SK=8192, CH=2048, NSUB=16, FGDIV=4, QKP=4, qk_subs=None, sm_sub=None, pv_plan=None,
                interpret=False, bounds=True, oproj_sub=0, paced=True):
    W = min(4096, max(256, SK // 4))
    assert SK % CH == 0 and W % CH == 0
    NCA, NCB = SK // CH, W // CH
    NA, NBs = B * HKV * NCA, B * HKV * NCB
    NSTEP = NA + NBs
    R = 2 * CH
    PR = R // NSUB
    FG = PR // FGDIV
    BG = PR - FG
    BGR = NSUB * BG
    assert BGR >= CH
    VB = BGR - CH
    lo, hi = (LO, HI) if paced else (0, 0)

    def avail(rows):
        return -(-rows // BG) - 1
    QR = CH // QKP
    if qk_subs is None:
        qk_subs = [avail((j + 1) * QR) for j in range(QKP)]
    for j in range(QKP):
        assert qk_subs[j] >= avail((j + 1) * QR)
    if sm_sub is None:
        sm_sub = qk_subs[-1] + 1
    if pv_plan is None:
        half = VB // 2
        pv_plan = [(sm_sub + 1, VB, CH), (max(sm_sub + 2, avail(CH + half)), 0, half), (NSUB - 1, half, VB)]
    for s, a, b_ in pv_plan:
        assert s > sm_sub or s == sm_sub
        if a < VB:
            assert b_ <= VB and s >= avail(CH + b_)
    TAIL0 = F - 2 * REP * DH
    TAIL1 = F - REP * DH
    NRT = D // 8

    def kernel(ax, ak, av, awq, awoT, bx, bk, bv, bwq, bwoT, o_ref,
               kv, wq_buf, wo_buf, x_buf, x8_s, q_s, o_s, out_s,
               bsem, fsem, wsem, msem):
        cp = pltpu.make_async_copy

        def kv_src(phase, j, r0, n):
            nc = NCA if phase == 0 else NCB
            if nc > 1:
                c = j % nc
                hb = j // nc
            else:
                c, hb = 0, j
            b = hb % B
            h = hb // B
            base = (0 if phase == 0 else SK - W) + c * CH
            if r0 < CH:
                src, off = (ak, bk)[phase], r0
            else:
                src, off = (av, bv)[phase], r0 - CH
            row = base + off
            if not isinstance(row, int):
                row = pl.multiple_of(row, 8)
            return src.at[b, h, pl.ds(row, n), :]

        def kv_bg_start(phase, j, slot, sub):
            r0, r1 = sub * BG, (sub + 1) * BG
            cuts = [r0, r1] if not (r0 < CH < r1) else [r0, CH, r1]
            for a, b_ in zip(cuts[:-1], cuts[1:]):
                cp(kv_src(phase, j, a, b_ - a), kv.at[slot, pl.ds(a, b_ - a), :], bsem.at[slot * NSUB + sub]).start(priority=lo)

        def kv_bg_wait(slot, sub):
            d = kv.at[slot, pl.ds(sub * BG, BG), :]
            cp(d, d, bsem.at[slot * NSUB + sub]).wait()

        def kv_fg_start(phase, j, slot, sub):
            r0 = BGR + sub * FG
            cp(kv_src(phase, j, r0, FG), kv.at[slot, pl.ds(r0, FG), :], fsem.at[slot]).start(priority=hi)

        def kv_fg_wait(slot):
            d = kv.at[slot, pl.ds(BGR, R - BGR), :]
            cp(d, d, fsem.at[slot]).wait()

        NW = 32
        w_bg = []
        for m, w in ((0, awq), (1, bwq)):
            for i in range(NRT):
                w_bg.append((w.at[pl.ds(i * 8, 8), :], wq_buf.at[m, pl.ds(i * 8, 8), :]))
        NBH = 24
        for i in range(NBH):
            w_bg.append((bwoT.at[pl.ds(i * 16, 16), pl.ds(0, TAIL0)], wo_buf.at[1, pl.ds(i * 16, 16), pl.ds(0, TAIL0)]))
        w_fg = []
        for i in range(NRT):
            for hf in range(2):
                w_fg.append(functools.partial(
                    lambda i, hf: cp(awoT.at[pl.ds(i * 8, 8), pl.ds(hf * (F // 2), F // 2)],
                                     wo_buf.at[0, pl.ds(i * 8, 8), pl.ds(hf * (F // 2), F // 2)], msem.at[0]).start(priority=hi), i, hf))
        for i in range(NBH * 2, NRT):
            w_fg.append(functools.partial(
                lambda i: cp(bwoT.at[pl.ds(i * 8, 8), pl.ds(0, TAIL0)], wo_buf.at[1, pl.ds(i * 8, 8), pl.ds(0, TAIL0)], msem.at[1]).start(priority=hi), i))
        for s in range(NSUB):
            w_fg.append(functools.partial(kv_fg_start, 0, 0, 0, s))
        NWS = len(w_bg)
        assert len(w_fg) <= NWS, (len(w_fg), NWS)

        def w_bg_copy(i):
            return cp(w_bg[i][0], w_bg[i][1], wsem.at[i % NW])

        DEPTH = NSUB
        for i in range(2):
            w_bg_copy(i).start(priority=lo)
        cp_xa = cp(ax, x_buf.at[0], msem.at[2])
        cp_xb = cp(bx, x_buf.at[1], msem.at[3])
        cp_xa.start(priority=hi)
        cp_xb.start(priority=hi)
        for i in range(2, DEPTH):
            w_bg_copy(i).start(priority=lo)

        q_s[...] = jnp.zeros(q_s.shape, q_s.dtype)
        o_s[...] = jnp.zeros(o_s.shape, o_s.dtype)
        x8_s[...] = jnp.zeros(x8_s.shape, x8_s.dtype)
        cp_xa.wait()
        cp_xb.wait()
        for ph in range(2):
            x8_s[ph, 0:B, :] = x_buf[ph].astype(jnp.float32)

        def qproj(ph):
            x8 = x8_s[ph].astype(jnp.bfloat16)
            q_all = lax.dot_general(x8, wq_buf[ph], NN, preferred_element_type=jnp.float32)
            q_all = q_all.astype(jnp.bfloat16).astype(jnp.float32) * (DH ** -0.5)
            for h in range(HKV):
                for b in range(B):
                    for r in range(REP):
                        col = (h * REP + r) * DH
                        q_s[ph * HKV * B + h * B + b, r:r + 1, :] = q_all[b:b + 1, col:col + DH]

        for i in range(NWS):
            w_bg_copy(i).wait()
            if i < len(w_fg):
                w_fg[i]()
            if i + DEPTH < NWS:
                w_bg_copy(i + DEPTH).start(priority=lo)
            else:
                kv_bg_start(0, 0, 0, i + DEPTH - NWS)
            if i == NRT - 1:
                qproj(0)
            if i == 2 * NRT - 1:
                qproj(1)

        NT6 = D // 32
        def t6_start(i):
            cp(bwoT.at[pl.ds(i * 32, 32), pl.ds(TAIL0, TAIL1 - TAIL0)], wo_buf.at[1, pl.ds(i * 32, 32), pl.ds(TAIL0, TAIL1 - TAIL0)], msem.at[4]).start(priority=hi)
        def t6_wait():
            d = wo_buf.at[1, :, pl.ds(TAIL0, TAIL1 - TAIL0)]
            cp(d, d, msem.at[4]).wait()
        NT7 = (F - TAIL1) // 128
        t7 = [cp(bwoT.at[:, pl.ds(TAIL1 + i * 128, 128)], wo_buf.at[1, :, pl.ds(TAIL1 + i * 128, 128)], msem.at[5 + i]) for i in range(NT7)]

        def oproj(phase, c0, c1):
            res = None
            c = c0
            while c < c1:
                hq = c // DH
                a = c - hq * DH
                e = min(DH, c1 - hq * DH)
                lhs = o_s[phase * HQ + hq, :, a:e].astype(jnp.bfloat16)
                part = lax.dot_general(lhs, wo_buf[phase, :, c:hq * DH + e], NT, preferred_element_type=jnp.float32)
                res = part if res is None else res + part
                c = hq * DH + e
            return res

        op_parts = []
        for g in range(4):
            op_parts.append((NA + 1 + g, 0, g * 1024, (g + 1) * 1024, g == 0))
        tb = NSTEP - 2 * B * NCB
        for g in range(3):
            op_parts.append((tb + g, 1, g * 1024, (g + 1) * 1024, g == 0))
        assert tb + 2 <= NSTEP - 2 and NA + 4 < tb

        def run_op_part(phase, c0, c1, first):
            if first:
                if phase == 0:
                    cp(wo_buf.at[0], wo_buf.at[0], msem.at[0]).wait()
                    out_s[0] = oproj(0, c0, c1)
                else:
                    d = wo_buf.at[1, pl.ds(NBH * 16, D - NBH * 16), pl.ds(0, TAIL0)]
                    cp(d, d, msem.at[1]).wait()
                    out_s[1] = oproj(1, c0, c1)
            else:
                out_s[phase] = out_s[phase] + oproj(phase, c0, c1)

        def step(t, carry, nxt):
            m, lvec, acc = carry
            static = isinstance(t, int)
            slot = t % 2
            nslot = 1 - slot
            if static:
                ph = 0 if t < NA else 1
                j = t if ph == 0 else t - NA
                nc = NCA if ph == 0 else NCB
                hb, first, last = j // nc, j % nc == 0, j % nc == nc - 1
            else:
                isa = t < NA
                ph = jnp.where(isa, 0, 1)
                hb = jnp.where(isa, t // NCA, (t - NA) // NCB)
                c = jnp.where(isa, t % NCA, (t - NA) % NCB)
                first = c == 0
                last = c == jnp.where(isa, NCA - 1, NCB - 1)
            qi = ph * (HKV * B) + hb
            jn = t + 1 if nxt == 0 else t + 1 - NA
            q = q_s[qi].astype(jnp.bfloat16)
            m = jnp.where(first, -jnp.inf, m)
            lvec = jnp.where(first, 0.0, lvec)
            acc = jnp.where(first, 0.0, acc)
            ss = [None] * QKP
            p = None
            fg_waited = False
            for sub in range(NSUB):
                kv_bg_wait(slot, sub)
                if nxt in (0, 1):
                    kv_fg_start(nxt, jn, nslot, sub)
                    kv_bg_start(nxt, jn, nslot, sub)
                else:
                    if sub < NT6:
                        t6_start(sub)
                    if sub < NT7:
                        t7[sub].start(priority=lo)
                if sub == oproj_sub and nxt == 1:
                    for (tt, php, c0, c1, fst) in op_parts:
                        pl.when(t == tt)(functools.partial(run_op_part, php, c0, c1, fst))
                for jq in range(QKP):
                    if qk_subs[jq] == sub:
                        ss[jq] = lax.dot_general(q, kv[slot, pl.ds(jq * QR, QR), :], NT, preferred_element_type=jnp.float32)
                if sub == sm_sub:
                    s = jnp.concatenate(ss, axis=1)
                    m_new = jnp.maximum(m, jnp.max(s, axis=-1, keepdims=True))
                    alpha = jnp.exp(m - m_new)
                    m = m_new
                    pf = jnp.exp(s - m)
                    lsum = pf[:, 0:128]
                    for k in range(1, CH // 128):
                        lsum = lsum + pf[:, k * 128:(k + 1) * 128]
                    lvec = lvec * alpha + lsum
                    acc = acc * alpha
                    p = pf.astype(jnp.bfloat16)
                for (ps, a, b_) in pv_plan:
                    if ps == sub:
                        if a >= VB and not fg_waited:
                            kv_fg_wait(slot)
                            fg_waited = True
                        acc = acc + lax.dot_general(p[:, a:b_], kv[slot, pl.ds(CH + a, b_ - a), :], NN, preferred_element_type=jnp.float32)
            assert fg_waited

            def fin():
                o = acc / jnp.sum(lvec, axis=-1, keepdims=True)
                b = hb % B
                h = hb // B
                for r in range(REP):
                    o_s[ph * HQ + h * REP + r, pl.ds(b, 1), :] = o[r:r + 1, :]
            if static:
                if last:
                    fin()
            else:
                pl.when(last)(fin)
            return m, lvec, acc

        init = (jnp.full((8, 1), -jnp.inf, jnp.float32), jnp.zeros((8, 128), jnp.float32), jnp.zeros((8, DH), jnp.float32))
        carry = lax.fori_loop(0, NA - 1, lambda t, c: step(t, c, 0), init)
        carry = lax.fori_loop(NA - 1, NSTEP - 1, lambda t, c: step(t, c, 1), carry)
        o_ref[:, 0:D] = out_s[0, 0:B, :].astype(o_ref.dtype)
        carry = step(NSTEP - 1, carry, 2)
        t6_wait()
        outb = out_s[1] + oproj(1, TAIL0, TAIL1)
        for i in range(NT7):
            t7[i].wait()
            outb = outb + oproj(1, TAIL1 + i * 128, TAIL1 + (i + 1) * 128)
        o_ref[:, D:2 * D] = outb[0:B, :].astype(o_ref.dtype)

    @jax.jit
    def f(A_x, A_k_cache, A_v_cache, A_wq, A_wo, B_x, B_k_cache, B_v_cache, B_wq, B_wo):
        hbm = pl.BlockSpec(memory_space=pltpu.HBM)
        out = pl.pallas_call(
            kernel,
            out_shape=jax.ShapeDtypeStruct((B, 2 * D), jnp.bfloat16),
            in_specs=[hbm] * 10,
            out_specs=pl.BlockSpec(memory_space=pltpu.VMEM),
            scratch_shapes=[
                pltpu.VMEM((2, R, DH), jnp.bfloat16),
                pltpu.VMEM((2, D, F), jnp.bfloat16),
                pltpu.VMEM((2, D, F), jnp.bfloat16),
                pltpu.VMEM((2, B, D), jnp.bfloat16),
                pltpu.VMEM((2, 8, D), jnp.float32),
                pltpu.VMEM((2 * HKV * B, 8, DH), jnp.float32),
                pltpu.VMEM((2 * HQ, 8, DH), jnp.float32),
                pltpu.VMEM((2, 8, D), jnp.float32),
                pltpu.SemaphoreType.DMA((2 * NSUB,)),
                pltpu.SemaphoreType.DMA((2,)),
                pltpu.SemaphoreType.DMA((32,)),
                pltpu.SemaphoreType.DMA((9,)),
            ],
            compiler_params=pltpu.CompilerParams(vmem_limit_bytes=64 * 1024 * 1024, disable_bounds_checks=not bounds),
            interpret=interpret,
        )(A_x.reshape(B, D), A_k_cache, A_v_cache, A_wq, A_wo.T,
          B_x.reshape(B, D), B_k_cache, B_v_cache, B_wq, B_wo.T)
        return out.reshape(B, 1, 2 * D)
    return f


_impl = make_kernel()


@jax.jit
def pallas_concat_heads__gqa_block_cached__sliding_block_cached__decode_kernel(
    A_x, A_k_cache, A_v_cache, A_wq, A_wo, B_x, B_k_cache, B_v_cache, B_wq, B_wo):
    return _impl(A_x, A_k_cache, A_v_cache, A_wq, A_wo, B_x, B_k_cache, B_v_cache, B_wq, B_wo)
```

```python
import functools
import jax
import jax.numpy as jnp
from jax import lax
from jax.experimental import pallas as pl
from jax.experimental.pallas import tpu as pltpu

NT = (((1,), (1,)), ((), ()))
NN = (((1,), (0,)), ((), ()))

B, D = 2, 448
HQ, HKV, DH = 16, 8, 256
REP = HQ // HKV
F = HQ * DH
LO, HI = 1, 0
NSLOT = 3


def make_kernel(SK=8192, CH=2048, NSUB=16, FG=80, QKP=8, PVP=4, pv_subs=(0, 3, 6, 9), qk_subs=None, sm_sub=None,
                op_sub=13, last_pv=None, h6_sub=14, t6_rows=64, wpad=0, qsplit=4, t7_groups=(4, 3, 1), NF=2,
                interpret=False, checks=False, nocompute=None):
    W = min(4096, max(256, SK // 4))
    assert SK % CH == 0 and W % CH == 0
    NCA, NCB = SK // CH, W // CH
    NA, NBs = B * HKV * NCA, B * HKV * NCB
    NSTEP = NA + NBs
    R = 2 * CH
    PR = R // NSUB
    BG = PR - FG
    BGR = NSUB * BG
    assert BGR >= CH
    VB = BGR - CH

    def avail(rows):
        return -(-rows // BG) - 1
    QR = CH // QKP
    VR = CH // PVP
    if qk_subs is None:
        qk_subs = [avail((j + 1) * QR) for j in range(QKP)]
    for j in range(QKP):
        assert qk_subs[j] >= avail((j + 1) * QR)
    if sm_sub is None:
        sm_sub = qk_subs[-1] + 1
    assert max(pv_subs) < sm_sub and len(pv_subs) == PVP
    if last_pv is None:
        cut = (VB * 2 // 3) // 128 * 128 if VB >= 384 else VB // 2
        last_pv = [(sm_sub + 1, VB, CH), (max(sm_sub + 1, avail(CH + cut)), 0, cut), (NSUB - 1, cut, VB)]
    for s, a, b_ in last_pv:
        assert s >= sm_sub
        if a < VB:
            assert b_ <= VB and s >= avail(CH + b_)
    TAIL1 = F - NF * REP * DH
    TAIL0 = TAIL1 - REP * DH
    NRT = D // 8
    NT7 = (F - TAIL1) // 128
    FP = F + wpad

    def kernel(ax, ak, av, awq, awoT, bx, bk, bv, bwq, bwoT, o_ref,
               kv, wq_buf, wo_buf, wt_buf, x_buf, x8_s, q_s, o_s, out_s, s_s, p_s,
               bsem, fsem, wsem, msem):
        cp = pltpu.make_async_copy

        def kv_src(phase, j, r0, n):
            nc = NCA if phase == 0 else NCB
            if nc > 1:
                c, hb = j % nc, j // nc
            else:
                c, hb = 0, j
            b, h = hb % B, hb // B
            base = (0 if phase == 0 else SK - W) + c * CH
            if r0 < CH:
                src, off = (ak, bk)[phase], r0
            else:
                src, off = (av, bv)[phase], r0 - CH
            row = base + off
            if not isinstance(row, int):
                row = pl.multiple_of(row, 8)
            return src.at[b, h, pl.ds(row, n), :]

        def kv_bg_start(phase, j, slot, sub):
            r0, r1 = sub * BG, (sub + 1) * BG
            cuts = [r0, r1] if not (r0 < CH < r1) else [r0, CH, r1]
            for a, b_ in zip(cuts[:-1], cuts[1:]):
                cp(kv_src(phase, j, a, b_ - a), kv.at[slot, pl.ds(a, b_ - a), :], bsem.at[slot * NSUB + sub]).start(priority=LO)

        def kv_bg_wait(slot, sub):
            d = kv.at[slot, pl.ds(sub * BG, BG), :]
            cp(d, d, bsem.at[slot * NSUB + sub]).wait()

        def kv_fg_start(phase, j, slot, sub):
            r0 = BGR + sub * FG
            cp(kv_src(phase, j, r0, FG), kv.at[slot, pl.ds(r0, FG), :], fsem.at[slot]).start(priority=HI)

        def kv_fg_wait(slot):
            d = kv.at[slot, pl.ds(BGR, R - BGR), :]
            cp(d, d, fsem.at[slot]).wait()

        NW = 32
        w_bg = []
        for m, w in ((0, awq), (1, bwq)):
            for i in range(NRT):
                w_bg.append((w.at[pl.ds(i * 8, 8), :], wq_buf.at[m, pl.ds(i * 8, 8), pl.ds(0, F)]))
        NBH = 24
        for i in range(NBH):
            w_bg.append((bwoT.at[pl.ds(i * 16, 16), pl.ds(0, TAIL0)], wo_buf.at[1, pl.ds(i * 16, 16), pl.ds(0, TAIL0)]))
        w_fg = []
        def woa_start(i, hf):
            cols = pl.ds(hf * (F // 2), F // 2)
            cp(awoT.at[pl.ds(i * 8, 8), cols], wo_buf.at[0, pl.ds(i * 8, 8), cols], msem.at[0]).start(priority=HI)
        def wobh_start(i):
            cp(bwoT.at[pl.ds(i * 8, 8), pl.ds(0, TAIL0)], wo_buf.at[1, pl.ds(i * 8, 8), pl.ds(0, TAIL0)], msem.at[1]).start(priority=HI)
        for i in range(NRT):
            for hf in range(2):
                w_fg.append(functools.partial(woa_start, i, hf))
        for i in range(NBH * 2, NRT):
            w_fg.append(functools.partial(wobh_start, i))
        for s in range(NSUB):
            w_fg.append(functools.partial(kv_fg_start, 0, 0, 0, s))
        NWS = len(w_bg)
        assert len(w_fg) <= NWS, (len(w_fg), NWS)

        def w_bg_copy(i):
            return cp(w_bg[i][0], w_bg[i][1], wsem.at[i % NW])

        DEPTH = NSUB
        for i in range(2):
            w_bg_copy(i).start(priority=LO)
        cp_xa = cp(ax, x_buf.at[0], msem.at[2])
        cp_xb = cp(bx, x_buf.at[1], msem.at[3])
        cp_xa.start(priority=HI)
        cp_xb.start(priority=HI)
        for i in range(2, DEPTH):
            w_bg_copy(i).start(priority=LO)

        q_s[...] = jnp.zeros(q_s.shape, q_s.dtype)
        o_s[...] = jnp.zeros(o_s.shape, o_s.dtype)
        x8_s[...] = jnp.zeros(x8_s.shape, x8_s.dtype)
        cp_xa.wait()
        cp_xb.wait()
        for ph in range(2):
            x8_s[ph, 0:B, :] = x_buf[ph].astype(jnp.float32)

        def qproj(ph, part):
            if nocompute in ('all', 'loops'):
                return
            cw = F // qsplit
            x8 = x8_s[ph].astype(jnp.bfloat16)
            qa = lax.dot_general(x8, wq_buf[ph, :, part * cw:(part + 1) * cw], NN, preferred_element_type=jnp.float32)
            qa = qa.astype(jnp.bfloat16).astype(jnp.float32) * (DH ** -0.5)
            for hq in range(part * cw // DH, (part + 1) * cw // DH):
                h, r = hq // REP, hq % REP
                col = hq * DH - part * cw
                for b in range(B):
                    q_s[ph * HKV * B + h * B + b, r:r + 1, :] = qa[b:b + 1, col:col + DH]

        for i in range(NWS):
            w_bg_copy(i).wait()
            if i < len(w_fg):
                w_fg[i]()
            if i + DEPTH < NWS:
                w_bg_copy(i + DEPTH).start(priority=LO)
            else:
                kv_bg_start(0, 0, 0, i + DEPTH - NWS)
            for ph in range(2):
                k = i - ((ph + 1) * NRT - 1)
                if k >= 0 and k % 2 == 0 and k // 2 < qsplit:
                    qproj(ph, k // 2)

        NT6 = D // t6_rows
        def t6_start(i):
            rows, cols = pl.ds(i * t6_rows, t6_rows), pl.ds(TAIL0, TAIL1 - TAIL0)
            cp(bwoT.at[rows, cols], wo_buf.at[1, rows, cols], msem.at[4]).start(priority=HI)
        def t6_wait():
            d = wo_buf.at[1, :, pl.ds(TAIL0, TAIL1 - TAIL0)]
            cp(d, d, msem.at[4]).wait()
        t7 = [cp(bwoT.at[:, pl.ds(TAIL1 + i * 128, 128)], wt_buf.at[i], msem.at[5 + i]) for i in range(NT7)]

        def oproj(phase, c0, c1):
            if nocompute == 'all' or (nocompute == 'loops' and c0 < TAIL0) or (nocompute == 'tail' and c0 >= TAIL0):
                return x8_s[0]
            res = None
            for hq in range(c0 // DH, c1 // DH):
                lhs = o_s[phase * HQ + hq].astype(jnp.bfloat16)
                part = lax.dot_general(lhs, wo_buf[phase, :, hq * DH:(hq + 1) * DH], NT, preferred_element_type=jnp.float32)
                res = part if res is None else res + part
            return res

        def oproj_t7(i):
            if nocompute in ('all', 'tail'):
                return x8_s[0]
            c = TAIL1 + i * 128
            lhs = o_s[HQ + c // DH, :, (c % DH):(c % DH) + 128].astype(jnp.bfloat16)
            return lax.dot_general(lhs, wt_buf[i], NT, preferred_element_type=jnp.float32)

        op_parts = []
        for g in range(4):
            op_parts.append((NA + g, 0, g * 1024, (g + 1) * 1024, g == 0))
        tb = NSTEP - (NF + 1) * B * NCB
        for g in range(3):
            op_parts.append((tb + g, 1, g * 1024, min(TAIL0, (g + 1) * 1024), g == 0))
        assert tb + 2 <= NSTEP - 2 and NA + 3 < tb and op_sub > max(pv_subs)

        def run_op_part(phase, c0, c1, first):
            if first:
                if phase == 0:
                    d = wo_buf.at[0, :, pl.ds(0, F)]
                    cp(d, d, msem.at[0]).wait()
                else:
                    d = wo_buf.at[1, pl.ds(NBH * 16, D - NBH * 16), pl.ds(0, TAIL0)]
                    cp(d, d, msem.at[1]).wait()
                out_s[phase] = oproj(phase, c0, c1)
            else:
                out_s[phase] = out_s[phase] + oproj(phase, c0, c1)

        def chunk_info(u):
            if isinstance(u, int):
                ph = 0 if u < NA else 1
                j = u if ph == 0 else u - NA
                nc = NCA if ph == 0 else NCB
                return ph, j // nc, j % nc == 0, j % nc == nc - 1
            isa = u < NA
            ph = jnp.where(isa, 0, 1)
            hb = jnp.where(isa, u // NCA, (u - NA) // NCB)
            c = jnp.where(isa, u % NCA, (u - NA) % NCB)
            return ph, hb, c == 0, c == jnp.where(isa, NCA - 1, NCB - 1)

        def finalize(u, lvec, acc):
            ph, hb, _, last = chunk_info(u)
            def fin():
                o = acc / jnp.sum(lvec, axis=-1, keepdims=True)
                b, h = hb % B, hb // B
                for r in range(REP):
                    o_s[ph * HQ + h * REP + r, pl.ds(b, 1), :] = o[r:r + 1, :]
            if isinstance(u, int):
                if last:
                    fin()
            else:
                pl.when(last)(fin)

        def pv(slot, a, b_):
            return lax.dot_general(p_s[:, a:b_].astype(jnp.bfloat16), kv[slot, pl.ds(CH + a, b_ - a), :], NN,
                                   preferred_element_type=jnp.float32)

        def step(t, carry, nxt, lagged=True):
            nc_here = nocompute == 'all' or (nocompute == 'loops' and nxt != 2) or (nocompute == 'tail' and nxt == 2)
            m, lvec, acc = carry
            slot = t % NSLOT
            nslot = (t + 1) % NSLOT
            pslot = (t + 2) % NSLOT
            ph, hb, first, _ = chunk_info(t)
            jn = t + 1 if nxt == 0 else t + 1 - NA
            q = q_s[ph * (HKV * B) + hb].astype(jnp.bfloat16)
            mx = None
            outb = None
            for sub in range(NSUB):
                kv_bg_wait(slot, sub)
                if nxt in (0, 1):
                    kv_fg_start(nxt, jn, nslot, sub)
                    kv_bg_start(nxt, jn, nslot, sub)
                else:
                    if sub < NT6:
                        t6_start(sub)
                    if sub < NT7:
                        t7[sub].start(priority=LO)
                if lagged and sub in pv_subs:
                    k = pv_subs.index(sub)
                    if k == 0:
                        kv_fg_wait(pslot)
                    if not nc_here:
                        acc = acc + pv(pslot, k * VR, (k + 1) * VR)
                        if k == PVP - 1:
                            finalize(t - 1, lvec, acc)
                if sub == op_sub and nxt == 1:
                    for (tt, php, c0, c1, fst) in op_parts:
                        pl.when(t == tt)(functools.partial(run_op_part, php, c0, c1, fst))
                for jq in range(QKP):
                    if qk_subs[jq] == sub and not nc_here:
                        s = lax.dot_general(q, kv[slot, pl.ds(jq * QR, QR), :], NT, preferred_element_type=jnp.float32)
                        s_s[:, jq * QR:(jq + 1) * QR] = s
                        for k in range(QR // 128):
                            blk = s[:, k * 128:(k + 1) * 128]
                            mx = blk if mx is None else jnp.maximum(mx, blk)
                if sub == sm_sub and not nc_here:
                    m_old = jnp.where(first, -jnp.inf, m)
                    m = jnp.maximum(m_old, jnp.max(mx, axis=-1, keepdims=True))
                    alpha = jnp.exp(m_old - m)
                    pf = jnp.exp(s_s[...] - m)
                    p_s[...] = pf
                    lsum = pf[:, 0:128]
                    for k in range(1, CH // 128):
                        lsum = lsum + pf[:, k * 128:(k + 1) * 128]
                    lvec = jnp.where(first, 0.0, lvec * alpha) + lsum
                    acc = jnp.where(first, 0.0, acc * alpha)
                if nxt == 2:
                    for (ps, a, b_) in last_pv:
                        if ps == sub:
                            if a == VB:
                                kv_fg_wait(slot)
                            if not nc_here:
                                acc = acc + pv(slot, a, b_)
                    if sub == h6_sub:
                        t6_wait()
                        outb = out_s[1] + oproj(1, TAIL0, TAIL1)
            if nxt == 2:
                if not nc_here:
                    finalize(t, lvec, acc)
                return outb
            return m, lvec, acc

        init = (jnp.full((8, 1), -jnp.inf, jnp.float32), jnp.zeros((8, 128), jnp.float32), jnp.zeros((8, DH), jnp.float32))
        carry = step(0, init, 0, lagged=False)
        carry = lax.fori_loop(1, NA - 1, lambda t, c: step(t, c, 0), carry)
        carry = lax.fori_loop(NA - 1, NSTEP - 1, lambda t, c: step(t, c, 1), carry)
        o_ref[:, 0:D] = out_s[0, 0:B, :].astype(o_ref.dtype)
        outb = step(NSTEP - 1, carry, 2)
        assert sum(t7_groups) == NT7
        i0 = 0
        for g in t7_groups:
            for i in range(i0, i0 + g):
                t7[i].wait()
            for i in range(i0, i0 + g):
                outb = outb + oproj_t7(i)
            i0 += g
        o_ref[:, D:2 * D] = outb[0:B, :].astype(o_ref.dtype)

    @jax.jit
    def f(A_x, A_k_cache, A_v_cache, A_wq, A_wo, B_x, B_k_cache, B_v_cache, B_wq, B_wo):
        hbm = pl.BlockSpec(memory_space=pltpu.HBM)
        out = pl.pallas_call(
            kernel,
            out_shape=jax.ShapeDtypeStruct((B, 2 * D), jnp.bfloat16),
            in_specs=[hbm] * 10,
            out_specs=pl.BlockSpec(memory_space=pltpu.VMEM),
            scratch_shapes=[
                pltpu.VMEM((NSLOT, R, DH), jnp.bfloat16),
                pltpu.VMEM((2, D, FP), jnp.bfloat16),
                pltpu.VMEM((2, D, FP), jnp.bfloat16),
                pltpu.VMEM((NT7, D, 128), jnp.bfloat16),
                pltpu.VMEM((2, B, D), jnp.bfloat16),
                pltpu.VMEM((2, 8, D), jnp.float32),
                pltpu.VMEM((2 * HKV * B, 8, DH), jnp.float32),
                pltpu.VMEM((2 * HQ, 8, DH), jnp.float32),
                pltpu.VMEM((2, 8, D), jnp.float32),
                pltpu.VMEM((8, CH), jnp.float32),
                pltpu.VMEM((8, CH), jnp.float32),
                pltpu.SemaphoreType.DMA((NSLOT * NSUB,)),
                pltpu.SemaphoreType.DMA((NSLOT,)),
                pltpu.SemaphoreType.DMA((32,)),
                pltpu.SemaphoreType.DMA((5 + NT7,)),
            ],
            compiler_params=pltpu.CompilerParams(vmem_limit_bytes=64 * 1024 * 1024, disable_bounds_checks=not checks,
                                                 disable_semaphore_checks=not checks),
            interpret=interpret,
        )(A_x.reshape(B, D), A_k_cache, A_v_cache, A_wq, A_wo.T,
          B_x.reshape(B, D), B_k_cache, B_v_cache, B_wq, B_wo.T)
        return out.reshape(B, 1, 2 * D)
    return f


_impl = make_kernel(h6_sub=10)


@jax.jit
def pallas_concat_heads__gqa_block_cached__sliding_block_cached__decode_kernel(
    A_x, A_k_cache, A_v_cache, A_wq, A_wo, B_x, B_k_cache, B_v_cache, B_wq, B_wo):
    return _impl(A_x, A_k_cache, A_v_cache, A_wq, A_wo, B_x, B_k_cache, B_v_cache, B_wq, B_wo)
```

```python
import functools

import jax
import jax.numpy as jnp
from jax import lax
from jax.experimental import pallas as pl
from jax.experimental.pallas import tpu as pltpu

NT = (((1,), (1,)), ((), ()))
NN = (((1,), (0,)), ((), ()))

B, D = 2, 448
HQ, HKV, DH = 16, 8, 256
REP = HQ // HKV
F = HQ * DH
LO, HI = 1, 0
NSLOT = 3
NSUB = 16


def make_kernel(SK=8192, CH=2048, FG=80, QKP=8, pv_subs=(0, 3, 6, 9), last_pv=None,
                interpret=False, checks=False):
    W = min(4096, max(256, SK // 4))
    assert SK % CH == 0 and W % CH == 0
    NCA, NCB = SK // CH, W // CH
    NA = B * HKV * NCA
    NSTEP = NA + B * HKV * NCB
    R = 2 * CH
    BG = R // NSUB - FG
    BGR = NSUB * BG
    VB = BGR - CH
    assert VB >= 0

    def avail(rows):
        return -(-rows // BG) - 1

    QR = CH // QKP
    PVP = len(pv_subs)
    VR = CH // PVP
    qk_subs = [avail((j + 1) * QR) for j in range(QKP)]
    sm_sub = qk_subs[-1] + 1
    op_sub = sm_sub + 1
    assert max(pv_subs) < sm_sub < NSUB - 1
    if last_pv is None:
        cut = VB * 2 // 3 // 128 * 128
        last_pv = [(sm_sub + 1, VB, CH), (avail(CH + cut), 0, cut), (NSUB - 1, cut, VB)]
    for s, a, b_ in last_pv:
        assert s > sm_sub and (a == VB or (b_ <= VB and s >= avail(CH + b_)))
    GW = REP * DH
    TAIL1 = F - 2 * GW
    TAIL0 = TAIL1 - GW
    NSLAB = (F - TAIL1) // 128
    SLAB_GROUPS = (4, 2, 2)
    assert sum(SLAB_GROUPS) == NSLAB
    NRT = D // 8
    SH = D % 128
    T6R = 32
    NT6 = D // T6R
    NBH = 24
    NW = 2 * NSUB

    def kernel(ax, ak, av, awq, awoT, bx, bk, bv, bwq, bwoT, o_ref,
               kv, wq_buf, wo_buf, wt_buf, x_buf, x8_s, q_s, o_s, out_s, s_s, p_s,
               bsem, fsem, wsem, msem):
        cp = pltpu.make_async_copy

        def wait_region(dst, sem):
            cp(dst, dst, sem).wait()

        def kv_src(phase, j, r0, n):
            nc = NCA if phase == 0 else NCB
            c, hb = (j % nc, j // nc) if nc > 1 else (0, j)
            b, h = hb % B, hb // B
            base = (0 if phase == 0 else SK - W) + c * CH
            if r0 < CH:
                src, off = (ak, bk)[phase], r0
            else:
                src, off = (av, bv)[phase], r0 - CH
            row = base + off
            if not isinstance(row, int):
                row = pl.multiple_of(row, 8)
            return src.at[b, h, pl.ds(row, n), :]

        def kv_bg_start(phase, j, slot, sub):
            r0, r1 = sub * BG, (sub + 1) * BG
            cuts = [r0, CH, r1] if r0 < CH < r1 else [r0, r1]
            for a, b_ in zip(cuts[:-1], cuts[1:]):
                cp(kv_src(phase, j, a, b_ - a), kv.at[slot, pl.ds(a, b_ - a), :],
                   bsem.at[slot * NSUB + sub]).start(priority=LO)

        def kv_bg_wait(slot, sub):
            wait_region(kv.at[slot, pl.ds(sub * BG, BG), :], bsem.at[slot * NSUB + sub])

        def kv_fg_start(phase, j, slot, sub):
            r0 = BGR + sub * FG
            cp(kv_src(phase, j, r0, FG), kv.at[slot, pl.ds(r0, FG), :], fsem.at[slot]).start(priority=HI)

        def kv_fg_wait(slot):
            wait_region(kv.at[slot, pl.ds(BGR, R - BGR), :], fsem.at[slot])

        head = pl.ds(0, TAIL0)
        w_bg = []
        for m, w in ((0, awq), (1, bwq)):
            for i in range(NRT):
                w_bg.append((w.at[pl.ds(i * 8, 8), :], wq_buf.at[m, pl.ds(i * 8, 8), :]))
        for i in range(NBH):
            w_bg.append((bwoT.at[pl.ds(i * 16, 16), head], wo_buf.at[1, pl.ds(i * 16, 16), head]))

        def woa_start(i, k):
            rows, cols = pl.ds(i * 8, 8), pl.ds(k * (F // 2), F // 2)
            cp(awoT.at[rows, cols], wo_buf.at[0, rows, cols], msem.at[0]).start(priority=HI)

        def wob_head_start(i):
            rows = pl.ds(i * 8, 8)
            cp(bwoT.at[rows, head], wo_buf.at[1, rows, head], msem.at[1]).start(priority=HI)

        w_fg = [functools.partial(woa_start, i, k) for i in range(NRT) for k in range(2)]
        w_fg += [functools.partial(wob_head_start, i) for i in range(2 * NBH, NRT)]
        w_fg += [functools.partial(kv_fg_start, 0, 0, 0, s) for s in range(NSUB)]
        NWS = len(w_bg)
        assert len(w_fg) <= NWS

        def w_bg_copy(i):
            return cp(w_bg[i][0], w_bg[i][1], wsem.at[i % NW])

        for i in range(2):
            w_bg_copy(i).start(priority=LO)
        cp_xa = cp(ax, x_buf.at[0], msem.at[2])
        cp_xb = cp(bx, x_buf.at[1], msem.at[3])
        cp_xa.start(priority=HI)
        cp_xb.start(priority=HI)
        for i in range(2, NSUB):
            w_bg_copy(i).start(priority=LO)

        q_s[...] = jnp.zeros(q_s.shape, q_s.dtype)
        o_s[...] = jnp.zeros(o_s.shape, o_s.dtype)
        x8_s[...] = jnp.zeros(x8_s.shape, x8_s.dtype)
        wt_buf[:, 0:SH, :] = jnp.zeros((NSLAB, SH, 128), wt_buf.dtype)
        cp_xa.wait()
        cp_xb.wait()
        for ph in range(2):
            x8_s[ph, 0:B, :] = x_buf[ph].astype(jnp.float32)

        QSPLIT = 4

        def qproj(ph, part):
            cw = F // QSPLIT
            x8 = x8_s[ph].astype(jnp.bfloat16)
            qa = lax.dot_general(x8, wq_buf[ph, :, part * cw:(part + 1) * cw], NN,
                                 preferred_element_type=jnp.float32)
            qa = qa.astype(jnp.bfloat16).astype(jnp.float32) * (DH ** -0.5)
            for hq in range(part * cw // DH, (part + 1) * cw // DH):
                h, r = hq // REP, hq % REP
                col = hq * DH - part * cw
                for b in range(B):
                    q_s[ph * HKV * B + h * B + b, r:r + 1, :] = qa[b:b + 1, col:col + DH]

        for i in range(NWS):
            w_bg_copy(i).wait()
            if i < len(w_fg):
                w_fg[i]()
            if i + NSUB < NWS:
                w_bg_copy(i + NSUB).start(priority=LO)
            else:
                kv_bg_start(0, 0, 0, i + NSUB - NWS)
            for ph in range(2):
                k = i - ((ph + 1) * NRT - 1)
                if k >= 0 and k % 2 == 0 and k // 2 < QSPLIT:
                    qproj(ph, k // 2)

        mid = pl.ds(TAIL0, TAIL1 - TAIL0)

        def mid_start(i):
            rows = pl.ds(i * T6R, T6R)
            cp(bwoT.at[rows, mid], wo_buf.at[1, rows, mid], msem.at[4]).start(priority=HI)

        slabs = [cp(bwoT.at[:, pl.ds(TAIL1 + i * 128, 128)], wt_buf.at[i, pl.ds(SH, D), :], msem.at[5 + i])
                 for i in range(NSLAB)]

        def oproj(phase, c0, c1):
            res = None
            for hq in range(c0 // DH, c1 // DH):
                lhs = o_s[phase * HQ + hq].astype(jnp.bfloat16)
                part = lax.dot_general(lhs, wo_buf[phase, :, hq * DH:(hq + 1) * DH], NT,
                                       preferred_element_type=jnp.float32)
                res = part if res is None else res + part
            return res

        def oproj_slab(i):
            c = TAIL1 + i * 128
            lhs = o_s[HQ + c // DH, :, (c % DH):(c % DH) + 128].astype(jnp.bfloat16)
            return lax.dot_general(lhs, wt_buf[i], NT, preferred_element_type=jnp.float32)

        op_parts = [(NA + g, 0, g * 1024, (g + 1) * 1024, g == 0) for g in range(F // 1024)]
        tb = NA + (TAIL0 // GW) * B * NCB
        op_parts += [(tb + g, 1, c0, min(TAIL0, c0 + 1024), g == 0) for g, c0 in enumerate(range(0, TAIL0, 1024))]
        assert NA + F // 1024 <= tb and max(p[0] for p in op_parts) <= NSTEP - 2

        def run_op_part(phase, c0, c1, first):
            if not first:
                out_s[phase] = out_s[phase] + oproj(phase, c0, c1)
                return
            if phase == 0:
                wait_region(wo_buf.at[0], msem.at[0])
            else:
                wait_region(wo_buf.at[1, pl.ds(NBH * 16, D - NBH * 16), head], msem.at[1])
            out_s[phase] = oproj(phase, c0, c1)

        def chunk_info(u):
            if isinstance(u, int):
                ph = 0 if u < NA else 1
                j, nc = (u, NCA) if ph == 0 else (u - NA, NCB)
                return ph, j // nc, j % nc == 0, j % nc == nc - 1
            isa = u < NA
            c = jnp.where(isa, u % NCA, (u - NA) % NCB)
            return (jnp.where(isa, 0, 1), jnp.where(isa, u // NCA, (u - NA) // NCB),
                    c == 0, c == jnp.where(isa, NCA - 1, NCB - 1))

        def finalize(u, lvec, acc):
            ph, hb, _, last = chunk_info(u)

            def fin():
                o = acc / jnp.sum(lvec, axis=-1, keepdims=True)
                b, h = hb % B, hb // B
                for r in range(REP):
                    o_s[ph * HQ + h * REP + r, pl.ds(b, 1), :] = o[r:r + 1, :]

            if isinstance(u, int):
                if last:
                    fin()
            else:
                pl.when(last)(fin)

        def pv(slot, a, b_):
            return lax.dot_general(p_s[:, a:b_].astype(jnp.bfloat16), kv[slot, pl.ds(CH + a, b_ - a), :], NN,
                                   preferred_element_type=jnp.float32)

        def step(t, carry, nxt, lagged=True):
            m, lvec, acc = carry
            slot, nslot, pslot = t % NSLOT, (t + 1) % NSLOT, (t + 2) % NSLOT
            ph, hb, first, _ = chunk_info(t)
            jn = t + 1 if nxt == 0 else t + 1 - NA
            q = q_s[ph * (HKV * B) + hb].astype(jnp.bfloat16)
            mx = None
            for sub in range(NSUB):
                kv_bg_wait(slot, sub)
                if nxt in (0, 1):
                    kv_fg_start(nxt, jn, nslot, sub)
                    kv_bg_start(nxt, jn, nslot, sub)
                else:
                    if sub < NT6:
                        mid_start(sub)
                    if sub < NSLAB:
                        slabs[sub].start(priority=LO)
                if lagged and sub in pv_subs:
                    k = pv_subs.index(sub)
                    if k == 0:
                        kv_fg_wait(pslot)
                    acc = acc + pv(pslot, k * VR, (k + 1) * VR)
                    if k == PVP - 1:
                        finalize(t - 1, lvec, acc)
                if sub == op_sub and nxt == 1:
                    for (tt, php, c0, c1, fst) in op_parts:
                        pl.when(t == tt)(functools.partial(run_op_part, php, c0, c1, fst))
                for jq in range(QKP):
                    if qk_subs[jq] == sub:
                        s = lax.dot_general(q, kv[slot, pl.ds(jq * QR, QR), :], NT,
                                            preferred_element_type=jnp.float32)
                        s_s[:, jq * QR:(jq + 1) * QR] = s
                        for k in range(QR // 128):
                            blk = s[:, k * 128:(k + 1) * 128]
                            mx = blk if mx is None else jnp.maximum(mx, blk)
                if sub == sm_sub:
                    m_old = jnp.where(first, -jnp.inf, m)
                    m = jnp.maximum(m_old, jnp.max(mx, axis=-1, keepdims=True))
                    alpha = jnp.exp(m_old - m)
                    p = jnp.exp(s_s[...] - m)
                    p_s[...] = p
                    lsum = p[:, 0:128]
                    for k in range(1, CH // 128):
                        lsum = lsum + p[:, k * 128:(k + 1) * 128]
                    lvec = jnp.where(first, 0.0, lvec * alpha) + lsum
                    acc = jnp.where(first, 0.0, acc * alpha)
                if nxt == 2:
                    for (ps, a, b_) in last_pv:
                        if ps == sub:
                            if a == VB:
                                kv_fg_wait(slot)
                            acc = acc + pv(slot, a, b_)
            return m, lvec, acc

        carry = (jnp.full((8, 1), -jnp.inf, jnp.float32), jnp.zeros((8, 128), jnp.float32),
                 jnp.zeros((8, DH), jnp.float32))
        carry = step(0, carry, 0, lagged=False)
        carry = lax.fori_loop(1, NA - 1, lambda t, c: step(t, c, 0), carry)
        carry = lax.fori_loop(NA - 1, NSTEP - 1, lambda t, c: step(t, c, 1), carry)
        o_ref[:, 0:D] = out_s[0, 0:B, :].astype(o_ref.dtype)
        _, lvec, acc = step(NSTEP - 1, carry, 2)
        wait_region(wo_buf.at[1, :, mid], msem.at[4])
        outb = out_s[1] + oproj(1, TAIL0, TAIL1)
        outb = jnp.concatenate([jnp.zeros((8, SH), jnp.float32), outb], axis=1)
        finalize(NSTEP - 1, lvec, acc)
        i0 = 0
        for g in SLAB_GROUPS:
            for i in range(i0, i0 + g):
                slabs[i].wait()
            for i in range(i0, i0 + g):
                outb = outb + oproj_slab(i)
            i0 += g
        o_ref[:, D:2 * D] = outb[0:B, SH:SH + D].astype(o_ref.dtype)

    def f(A_x, A_k_cache, A_v_cache, A_wq, A_wo, B_x, B_k_cache, B_v_cache, B_wq, B_wo):
        assert A_k_cache.shape == B_k_cache.shape == (B, HKV, SK, DH)
        assert A_wq.shape == (D, F) and A_wo.shape == (F, D) and A_x.shape == (B, 1, D)
        hbm = pl.BlockSpec(memory_space=pltpu.HBM)
        out = pl.pallas_call(
            kernel,
            out_shape=jax.ShapeDtypeStruct((B, 2 * D), A_x.dtype),
            in_specs=[hbm] * 10,
            out_specs=pl.BlockSpec(memory_space=pltpu.VMEM),
            scratch_shapes=[
                pltpu.VMEM((NSLOT, R, DH), jnp.bfloat16),
                pltpu.VMEM((2, D, F), jnp.bfloat16),
                pltpu.VMEM((2, D, F), jnp.bfloat16),
                pltpu.VMEM((NSLAB, SH + D, 128), jnp.bfloat16),
                pltpu.VMEM((2, B, D), jnp.bfloat16),
                pltpu.VMEM((2, 8, D), jnp.float32),
                pltpu.VMEM((2 * HKV * B, 8, DH), jnp.float32),
                pltpu.VMEM((2 * HQ, 8, DH), jnp.float32),
                pltpu.VMEM((2, 8, D), jnp.float32),
                pltpu.VMEM((8, CH), jnp.float32),
                pltpu.VMEM((8, CH), jnp.float32),
                pltpu.SemaphoreType.DMA((NSLOT * NSUB,)),
                pltpu.SemaphoreType.DMA((NSLOT,)),
                pltpu.SemaphoreType.DMA((NW,)),
                pltpu.SemaphoreType.DMA((5 + NSLAB,)),
            ],
            compiler_params=pltpu.CompilerParams(
                vmem_limit_bytes=64 * 1024 * 1024,
                disable_semaphore_checks=not checks),
            interpret=interpret,
        )(A_x.reshape(B, D), A_k_cache, A_v_cache, A_wq, A_wo.T,
          B_x.reshape(B, D), B_k_cache, B_v_cache, B_wq, B_wo.T)
        return out.reshape(B, 1, 2 * D)

    return jax.jit(f)


_impl = make_kernel()


@jax.jit
def pallas_concat_heads__gqa_block_cached__sliding_block_cached__decode_kernel(
    A_x, A_k_cache, A_v_cache, A_wq, A_wo, B_x, B_k_cache, B_v_cache, B_wq, B_wo):
    return _impl(A_x, A_k_cache, A_v_cache, A_wq, A_wo, B_x, B_k_cache, B_v_cache, B_wq, B_wo)
```

```python
import functools

import jax
import jax.numpy as jnp
from jax import lax
from jax.experimental import pallas as pl
from jax.experimental.pallas import tpu as pltpu

NT = (((1,), (1,)), ((), ()))
NN = (((1,), (0,)), ((), ()))

B, D = 2, 448
HQ, HKV, DH = 16, 8, 256
REP = HQ // HKV
F = HQ * DH
LO, HI = 1, 0
NSLOT = 3
NSUB = 16


def make_kernel(SK=8192, CH=2048, FG=96, QKP=8, pv_subs=(0, 2, 5, 8), fin_sub=10, op_sub=15, last_pv=None,
                interpret=False, checks=False):
    W = min(4096, max(256, SK // 4))
    assert SK % CH == 0 and W % CH == 0
    NCA, NCB = SK // CH, W // CH
    NA = B * HKV * NCA
    NSTEP = NA + B * HKV * NCB
    R = 2 * CH
    BG = R // NSUB - FG
    BGR = NSUB * BG
    VB = BGR - CH
    assert VB >= 0

    def avail(rows):
        return -(-rows // BG) - 1

    QR = CH // QKP
    PVP = len(pv_subs)
    VR = CH // PVP
    qk_subs = [avail((j + 1) * QR) for j in range(QKP)]
    sm_sub = qk_subs[-1] + 1
    assert max(pv_subs) <= fin_sub < min(sm_sub, op_sub) and max(sm_sub, op_sub) < NSUB
    OPC = 1024
    if last_pv is None:
        cut = VB * 2 // 3 // 128 * 128
        last_pv = [(sm_sub + 1, VB, CH), (avail(CH + cut), 0, cut), (NSUB - 1, cut, VB)]
    for s, a, b_ in last_pv:
        assert s >= sm_sub and (a == VB or (b_ <= VB and s >= avail(CH + b_)))
    GW = REP * DH
    TAIL1 = F - 2 * GW
    TAIL0 = TAIL1 - GW
    NSLAB = (F - TAIL1) // 128
    SLAB_GROUPS = (4, 2, 2)
    assert sum(SLAB_GROUPS) == NSLAB
    NRT = D // 8
    SH = D % 128
    T6R = 32
    NT6 = D // T6R
    NBH = 24
    NW = 2 * NSUB

    def kernel(ax, ak, av, awq, awoT, bx, bk, bv, bwq, bwoT, o_ref,
               kv, wq_buf, wo_buf, wt_buf, x_buf, x8_s, q_s, o_s, out_s, s_s, p_s,
               bsem, fsem, wsem, msem):
        cp = pltpu.make_async_copy

        def wait_region(dst, sem):
            cp(dst, dst, sem).wait()

        def kv_src(phase, j, r0, n):
            nc = NCA if phase == 0 else NCB
            c, hb = (j % nc, j // nc) if nc > 1 else (0, j)
            b, h = hb % B, hb // B
            base = (0 if phase == 0 else SK - W) + c * CH
            if r0 < CH:
                src, off = (ak, bk)[phase], r0
            else:
                src, off = (av, bv)[phase], r0 - CH
            row = base + off
            if not isinstance(row, int):
                row = pl.multiple_of(row, 8)
            return src.at[b, h, pl.ds(row, n), :]

        def kv_bg_start(phase, j, slot, sub):
            r0, r1 = sub * BG, (sub + 1) * BG
            cuts = [r0, CH, r1] if r0 < CH < r1 else [r0, r1]
            for a, b_ in zip(cuts[:-1], cuts[1:]):
                cp(kv_src(phase, j, a, b_ - a), kv.at[slot, pl.ds(a, b_ - a), :],
                   bsem.at[slot * NSUB + sub]).start(priority=LO)

        def kv_bg_wait(slot, sub):
            wait_region(kv.at[slot, pl.ds(sub * BG, BG), :], bsem.at[slot * NSUB + sub])

        def kv_fg_start(phase, j, slot, sub):
            r0 = BGR + sub * FG
            cp(kv_src(phase, j, r0, FG), kv.at[slot, pl.ds(r0, FG), :], fsem.at[slot]).start(priority=HI)

        def kv_fg_wait(slot):
            wait_region(kv.at[slot, pl.ds(BGR, R - BGR), :], fsem.at[slot])

        head = pl.ds(0, TAIL0)
        w_bg = []
        for m, w in ((0, awq), (1, bwq)):
            for i in range(NRT):
                w_bg.append((w.at[pl.ds(i * 8, 8), :], wq_buf.at[m, pl.ds(i * 8, 8), :]))
        for i in range(NBH):
            w_bg.append((bwoT.at[pl.ds(i * 16, 16), head], wo_buf.at[1, pl.ds(i * 16, 16), head]))

        def woa_start(i, k):
            rows, cols = pl.ds(i * 8, 8), pl.ds(k * (F // 2), F // 2)
            cp(awoT.at[rows, cols], wo_buf.at[0, rows, cols], msem.at[0]).start(priority=HI)

        def wob_head_start(i):
            rows = pl.ds(i * 8, 8)
            cp(bwoT.at[rows, head], wo_buf.at[1, rows, head], msem.at[1]).start(priority=HI)

        w_fg = [functools.partial(woa_start, i, k) for i in range(NRT) for k in range(2)]
        w_fg += [functools.partial(wob_head_start, i) for i in range(2 * NBH, NRT)]
        w_fg += [functools.partial(kv_fg_start, 0, 0, 0, s) for s in range(NSUB)]
        NWS = len(w_bg)
        assert len(w_fg) <= NWS

        def w_bg_copy(i):
            return cp(w_bg[i][0], w_bg[i][1], wsem.at[i % NW])

        for i in range(2):
            w_bg_copy(i).start(priority=LO)
        cp_xa = cp(ax, x_buf.at[0], msem.at[2])
        cp_xb = cp(bx, x_buf.at[1], msem.at[3])
        cp_xa.start(priority=HI)
        cp_xb.start(priority=HI)
        for i in range(2, NSUB):
            w_bg_copy(i).start(priority=LO)

        q_s[...] = jnp.zeros(q_s.shape, q_s.dtype)
        o_s[...] = jnp.zeros(o_s.shape, o_s.dtype)
        x8_s[...] = jnp.zeros(x8_s.shape, x8_s.dtype)
        wt_buf[:, 0:SH, :] = jnp.zeros((NSLAB, SH, 128), wt_buf.dtype)
        cp_xa.wait()
        cp_xb.wait()
        for ph in range(2):
            x8_s[ph, 0:B, :] = x_buf[ph].astype(jnp.float32)

        QSPLIT = 4

        def qproj(ph, part):
            cw = F // QSPLIT
            x8 = x8_s[ph].astype(jnp.bfloat16)
            qa = lax.dot_general(x8, wq_buf[ph, :, part * cw:(part + 1) * cw], NN,
                                 preferred_element_type=jnp.float32)
            qa = qa.astype(jnp.bfloat16).astype(jnp.float32) * (DH ** -0.5)
            for hq in range(part * cw // DH, (part + 1) * cw // DH):
                h, r = hq // REP, hq % REP
                col = hq * DH - part * cw
                for b in range(B):
                    q_s[ph * HKV * B + h * B + b, r:r + 1, :] = qa[b:b + 1, col:col + DH]

        for i in range(NWS):
            w_bg_copy(i).wait()
            if i < len(w_fg):
                w_fg[i]()
            if i + NSUB < NWS:
                w_bg_copy(i + NSUB).start(priority=LO)
            else:
                kv_bg_start(0, 0, 0, i + NSUB - NWS)
            for ph in range(2):
                k = i - ((ph + 1) * NRT - 1)
                if k >= 0 and k % 2 == 0 and k // 2 < QSPLIT:
                    qproj(ph, k // 2)

        mid = pl.ds(TAIL0, TAIL1 - TAIL0)

        def mid_start(i):
            rows = pl.ds(i * T6R, T6R)
            cp(bwoT.at[rows, mid], wo_buf.at[1, rows, mid], msem.at[4]).start(priority=HI)

        slabs = [cp(bwoT.at[:, pl.ds(TAIL1 + i * 128, 128)], wt_buf.at[i, pl.ds(SH, D), :], msem.at[5 + i])
                 for i in range(NSLAB)]

        def oproj(phase, c0, c1):
            res = None
            for hq in range(c0 // DH, c1 // DH):
                lhs = o_s[phase * HQ + hq].astype(jnp.bfloat16)
                part = lax.dot_general(lhs, wo_buf[phase, :, hq * DH:(hq + 1) * DH], NT,
                                       preferred_element_type=jnp.float32)
                res = part if res is None else res + part
            return res

        def oproj_slab(i):
            c = TAIL1 + i * 128
            lhs = o_s[HQ + c // DH, :, (c % DH):(c % DH) + 128].astype(jnp.bfloat16)
            return lax.dot_general(lhs, wt_buf[i], NT, preferred_element_type=jnp.float32)

        op_parts = [(NA + g, 0, g * OPC, (g + 1) * OPC, g == 0) for g in range(F // OPC)]
        tb = NA + (TAIL0 // GW) * B * NCB
        op_parts += [(tb + g, 1, c0, min(TAIL0, c0 + OPC), g == 0) for g, c0 in enumerate(range(0, TAIL0, OPC))]
        assert NA + F // OPC <= tb and max(p[0] for p in op_parts) <= NSTEP - 2

        def run_op_part(phase, c0, c1, first):
            if not first:
                out_s[phase] = out_s[phase] + oproj(phase, c0, c1)
                return
            if phase == 0:
                wait_region(wo_buf.at[0], msem.at[0])
            else:
                wait_region(wo_buf.at[1, pl.ds(NBH * 16, D - NBH * 16), head], msem.at[1])
            out_s[phase] = oproj(phase, c0, c1)

        def chunk_info(u):
            if isinstance(u, int):
                ph = 0 if u < NA else 1
                j, nc = (u, NCA) if ph == 0 else (u - NA, NCB)
                return ph, j // nc, j % nc == 0, j % nc == nc - 1
            isa = u < NA
            c = jnp.where(isa, u % NCA, (u - NA) % NCB)
            return (jnp.where(isa, 0, 1), jnp.where(isa, u // NCA, (u - NA) // NCB),
                    c == 0, c == jnp.where(isa, NCA - 1, NCB - 1))

        def finalize(u, lvec, acc):
            ph, hb, _, last = chunk_info(u)

            def fin():
                o = acc / jnp.sum(lvec, axis=-1, keepdims=True)
                b, h = hb % B, hb // B
                for r in range(REP):
                    o_s[ph * HQ + h * REP + r, pl.ds(b, 1), :] = o[r:r + 1, :]

            if isinstance(u, int):
                if last:
                    fin()
            else:
                pl.when(last)(fin)

        def pv(slot, a, b_):
            return lax.dot_general(p_s[:, a:b_].astype(jnp.bfloat16), kv[slot, pl.ds(CH + a, b_ - a), :], NN,
                                   preferred_element_type=jnp.float32)

        def step(t, carry, nxt, lagged=True):
            m, lvec, acc = carry
            slot, nslot, pslot = t % NSLOT, (t + 1) % NSLOT, (t + 2) % NSLOT
            ph, hb, first, _ = chunk_info(t)
            jn = t + 1 if nxt == 0 else t + 1 - NA
            q = q_s[ph * (HKV * B) + hb].astype(jnp.bfloat16)
            mx = None
            for sub in range(NSUB):
                kv_bg_wait(slot, sub)
                if nxt in (0, 1):
                    kv_fg_start(nxt, jn, nslot, sub)
                    kv_bg_start(nxt, jn, nslot, sub)
                else:
                    if sub < NT6:
                        mid_start(sub)
                    if sub < NSLAB:
                        slabs[sub].start(priority=LO)
                if lagged and sub in pv_subs:
                    k = pv_subs.index(sub)
                    if k == 0:
                        kv_fg_wait(pslot)
                    acc = acc + pv(pslot, k * VR, (k + 1) * VR)
                if lagged and sub == fin_sub:
                    finalize(t - 1, lvec, acc)
                if sub == op_sub and nxt == 1:
                    for (tt, php, c0, c1, fst) in op_parts:
                        pl.when(t == tt)(functools.partial(run_op_part, php, c0, c1, fst))
                for jq in range(QKP):
                    if qk_subs[jq] == sub:
                        s = lax.dot_general(q, kv[slot, pl.ds(jq * QR, QR), :], NT,
                                            preferred_element_type=jnp.float32)
                        s_s[:, jq * QR:(jq + 1) * QR] = s
                        for k in range(QR // 128):
                            blk = s[:, k * 128:(k + 1) * 128]
                            mx = blk if mx is None else jnp.maximum(mx, blk)
                if sub == sm_sub:
                    m_old = jnp.where(first, -jnp.inf, m)
                    m = jnp.maximum(m_old, jnp.max(mx, axis=-1, keepdims=True))
                    alpha = jnp.exp(m_old - m)
                    p = jnp.exp(s_s[...] - m)
                    p_s[...] = p
                    lsum = p[:, 0:128]
                    for k in range(1, CH // 128):
                        lsum = lsum + p[:, k * 128:(k + 1) * 128]
                    lvec = jnp.where(first, 0.0, lvec * alpha) + lsum
                    acc = jnp.where(first, 0.0, acc * alpha)
                if nxt == 2:
                    for (ps, a, b_) in last_pv:
                        if ps == sub:
                            if a == VB:
                                kv_fg_wait(slot)
                            acc = acc + pv(slot, a, b_)
            return m, lvec, acc

        carry = (jnp.full((8, 1), -jnp.inf, jnp.float32), jnp.zeros((8, 128), jnp.float32),
                 jnp.zeros((8, DH), jnp.float32))
        carry = step(0, carry, 0, lagged=False)
        carry = lax.fori_loop(1, NA - 1, lambda t, c: step(t, c, 0), carry)
        carry = lax.fori_loop(NA - 1, NSTEP - 1, lambda t, c: step(t, c, 1), carry)
        o_ref[:, 0:D] = out_s[0, 0:B, :].astype(o_ref.dtype)
        _, lvec, acc = step(NSTEP - 1, carry, 2)
        wait_region(wo_buf.at[1, :, mid], msem.at[4])
        outb = out_s[1] + oproj(1, TAIL0, TAIL1)
        outb = jnp.concatenate([jnp.zeros((8, SH), jnp.float32), outb], axis=1)
        finalize(NSTEP - 1, lvec, acc)
        i0 = 0
        for g in SLAB_GROUPS:
            for i in range(i0, i0 + g):
                slabs[i].wait()
            for i in range(i0, i0 + g):
                outb = outb + oproj_slab(i)
            i0 += g
        o_ref[:, D:2 * D] = outb[0:B, SH:SH + D].astype(o_ref.dtype)

    def f(A_x, A_k_cache, A_v_cache, A_wq, A_wo, B_x, B_k_cache, B_v_cache, B_wq, B_wo):
        assert A_k_cache.shape == B_k_cache.shape == (B, HKV, SK, DH)
        assert A_wq.shape == (D, F) and A_wo.shape == (F, D) and A_x.shape == (B, 1, D)
        hbm = pl.BlockSpec(memory_space=pltpu.HBM)
        out = pl.pallas_call(
            kernel,
            out_shape=jax.ShapeDtypeStruct((B, 2 * D), A_x.dtype),
            in_specs=[hbm] * 10,
            out_specs=pl.BlockSpec(memory_space=pltpu.VMEM),
            scratch_shapes=[
                pltpu.VMEM((NSLOT, R, DH), jnp.bfloat16),
                pltpu.VMEM((2, D, F), jnp.bfloat16),
                pltpu.VMEM((2, D, F), jnp.bfloat16),
                pltpu.VMEM((NSLAB, SH + D, 128), jnp.bfloat16),
                pltpu.VMEM((2, B, D), jnp.bfloat16),
                pltpu.VMEM((2, 8, D), jnp.float32),
                pltpu.VMEM((2 * HKV * B, 8, DH), jnp.float32),
                pltpu.VMEM((2 * HQ, 8, DH), jnp.float32),
                pltpu.VMEM((2, 8, D), jnp.float32),
                pltpu.VMEM((8, CH), jnp.float32),
                pltpu.VMEM((8, CH), jnp.float32),
                pltpu.SemaphoreType.DMA((NSLOT * NSUB,)),
                pltpu.SemaphoreType.DMA((NSLOT,)),
                pltpu.SemaphoreType.DMA((NW,)),
                pltpu.SemaphoreType.DMA((5 + NSLAB,)),
            ],
            compiler_params=pltpu.CompilerParams(
                vmem_limit_bytes=64 * 1024 * 1024,
                disable_semaphore_checks=not checks),
            interpret=interpret,
        )(A_x.reshape(B, D), A_k_cache, A_v_cache, A_wq, A_wo.T,
          B_x.reshape(B, D), B_k_cache, B_v_cache, B_wq, B_wo.T)
        return out.reshape(B, 1, 2 * D)

    return jax.jit(f)


_impl = make_kernel()


@jax.jit
def pallas_concat_heads__gqa_block_cached__sliding_block_cached__decode_kernel(
    A_x, A_k_cache, A_v_cache, A_wq, A_wo, B_x, B_k_cache, B_v_cache, B_wq, B_wo):
    return _impl(A_x, A_k_cache, A_v_cache, A_wq, A_wo, B_x, B_k_cache, B_v_cache, B_wq, B_wo)
```
